```python
import jax
import jax.numpy as jnp

def _softmax(x, axis=-1):
    return jax.nn.softmax(x, axis=axis)
def _gelu(x):
    return jax.nn.gelu(x, approximate=True)
def _silu(x):
    return jax.nn.silu(x)
def _sigmoid(x):
    return jax.nn.sigmoid(x)
def _layernorm(x, axis=-1, eps=1e-5):
    m = jnp.mean(x, axis=axis, keepdims=True)
    v = jnp.var(x, axis=axis, keepdims=True)
    return (x - m) / jnp.sqrt(v + eps)
def _scatter_add(tgt, idx, src, axis=0):
    return tgt.at[idx].add(src)
def _segment_sum(src, seg, n):
    return jax.ops.segment_sum(src, seg, n)
class _Rng:
    def __init__(self, key):
        self._k = key
    def _next(self):
        self._k, sub = jax.random.split(self._k)
        return sub
    def normal(self, shape):
        return jax.random.normal(self._next(), shape, dtype=jnp.bfloat16)
    def randint(self, lo, hi, shape):
        return jax.random.randint(self._next(), shape, lo, hi, dtype=jnp.int32)
    def uniform(self, shape, lo=0.0, hi=1.0):
        return jax.random.uniform(self._next(), shape, jnp.bfloat16, lo, hi)
    def permutation(self, n):
        return jax.random.permutation(self._next(), n)


kernel_name = 'recurrent_scan__sliding_block_cached__mixer_s_mlp__decode'

def setup_inputs():
    _rng = _Rng(jax.random.key(int.from_bytes(__import__("os").urandom(4), "little")))
    _w = (lambda a: (lambda t: t.astype(jnp.bfloat16) if jnp.issubdtype(t.dtype, jnp.floating) else t)(jnp.asarray(a)))
    def _A_setup():
        B, Sq, D = 1, 1, 512
        Hq, Hkv, Sk, Dh = 32, 32, 32768, 128
        assert Hq % Hkv == 0, (Hq, Hkv)
        return {
            "x": _w((lambda *s: _rng.normal(s) * 0.05)(B, Sq, D)),
            "k_cache": _w((lambda *s: _rng.normal(s) * 0.05)(B, Hkv, Sk, Dh)),
            "v_cache": _w((lambda *s: _rng.normal(s) * 0.05)(B, Hkv, Sk, Dh)),
            "wq": _w((lambda *s: _rng.normal(s) * 0.05)(D, Hq * Dh) * (D ** -0.5)),
            "wo": _w((lambda *s: _rng.normal(s) * 0.05)(Hq * Dh, D) * ((Hq * Dh) ** -0.5)),
        }
    _A_in = _A_setup()

    def _B_setup():
        B, S, D, F = 1, 1, 512, 1376
        return {
            "x":  _w((lambda *s: _rng.normal(s) * 0.05)(B, S, D)),
            "w1": _w((lambda *s: _rng.normal(s) * 0.05)(D, D) * (D ** -0.5)),
            "w2": _w((lambda *s: _rng.normal(s) * 0.05)(D, D) * (D ** -0.5)),
            "w3": _w((lambda *s: _rng.normal(s) * 0.05)(D, F) * (D ** -0.5)),
            "w4": _w((lambda *s: _rng.normal(s) * 0.05)(F, D) * (F ** -0.5)),
        }
    _B_in = _B_setup()

    return {
        "A_x": _A_in["x"],
        "A_k_cache": _A_in["k_cache"],
        "A_v_cache": _A_in["v_cache"],
        "A_wq": _A_in["wq"],
        "A_wo": _A_in["wo"],
        "B_x": _B_in["x"],
        "B_w1": _B_in["w1"],
        "B_w2": _B_in["w2"],
        "B_w3": _B_in["w3"],
        "B_w4": _B_in["w4"],
    }

def reference(A_x, A_k_cache, A_v_cache, A_wq, A_wo, B_x, B_w1, B_w2, B_w3, B_w4):
    def _A_ref(x, k_cache, v_cache, wq, wo):
        B, Sq, D = x.shape
        Hq, Dh = 32, 128
        Hkv, Sk = k_cache.shape[1], k_cache.shape[2]
        W = min(4096, max(256, Sk // 4))
        rep = Hq // Hkv
        q = (lambda x, *d: x.transpose(*d))((x @ wq).reshape(B, Sq, Hq, Dh), 0, 2, 1, 3)
        k = jnp.repeat(k_cache[:, :, Sk - W:, :], rep, axis=1)
        v = jnp.repeat(v_cache[:, :, Sk - W:, :], rep, axis=1)
        scores = jnp.einsum("bhqd,bhkd->bhqk", q, k) * (Dh ** -0.5)
        p = _softmax(scores, axis=-1)
        o = jnp.einsum("bhqk,bhkd->bhqd", p, v)
        return (lambda x, *d: x.transpose(*d))(o, 0, 2, 1, 3).reshape(B, Sq, Hq * Dh) @ wo

    def _B_ref(x, w1, w2, w3, w4):
        B, S, D = x.shape
        h = _gelu(_layernorm(x, axis=-1) @ w1)
        c = D // 4
        g0 = jnp.pad(h[:, :, 0*c:1*c], ((0, 0), (1, 0), (0, 0)))[:, :S, :]
        g1 = jnp.pad(h[:, :, 1*c:2*c], ((0, 0), (0, 1), (0, 0)))[:, 1:, :]
        g2 = jnp.pad(h[:, :, 2*c:3*c], ((0, 0), (2, 0), (0, 0)))[:, :S, :]
        g3 = jnp.pad(h[:, :, 3*c:   ], ((0, 0), (0, 2), (0, 0)))[:, 2:, :]
        hs = jnp.concatenate([g0, g1, g2, g3], axis=-1) @ w2
        x1 = x + hs
        h2 = _gelu(_layernorm(x1, axis=-1) @ w3) @ w4
        return x1 + h2

    x = A_x
    xn = _layernorm(x, axis=-1)
    s = _A_ref(xn, A_k_cache, A_v_cache, A_wq, A_wo)
    g = _silu(_B_ref(xn, B_w1, B_w2, B_w3, B_w4))
    return x + s * g
```

```python
import functools

import jax
import jax.numpy as jnp
from jax import lax
import jax.experimental.pallas as pl
import jax.experimental.pallas.tpu as pltpu

_EPS = 1e-5


def _layernorm(x):
    m = jnp.mean(x, axis=-1, keepdims=True)
    d = x - m
    v = jnp.mean(d * d, axis=-1, keepdims=True)
    return d * lax.rsqrt(v + _EPS)


def _kernel(x_hbm, k_hbm, v_hbm, wq_hbm, wo_hbm, w3_hbm, w4_hbm, o_ref,
            x_v, wq_v, wo_v, w3_v, w4_v, k_v, v_v, q_v, att_v,
            wsem, ksem, vsem, *, H, Dh, Sk, W, depth):
    bf16, f32 = jnp.bfloat16, jnp.float32

    def k_copy(h):
        return pltpu.make_async_copy(
            k_hbm.at[0, h, pl.ds(Sk - W, W), :], k_v.at[h], ksem.at[h])

    def v_copy(h):
        return pltpu.make_async_copy(
            v_hbm.at[0, h, pl.ds(Sk - W, W), :], v_v.at[h], vsem.at[h])

    x_cp = pltpu.make_async_copy(x_hbm, x_v, wsem.at[0])
    wq_cp = pltpu.make_async_copy(wq_hbm, wq_v, wsem.at[1])
    w3_cp = pltpu.make_async_copy(w3_hbm, w3_v, wsem.at[2])
    w4_cp = pltpu.make_async_copy(w4_hbm, w4_v, wsem.at[3])
    wo_cp = pltpu.make_async_copy(wo_hbm, wo_v, wsem.at[4])

    x_cp.start()
    wq_cp.start()
    w3_cp.start()
    w4_cp.start()
    wo_cp.start()
    for h in range(min(depth, H)):
        k_copy(h).start()
        v_copy(h).start()

    x_cp.wait()
    x = x_v[...].astype(f32)
    xn = _layernorm(x).astype(bf16)

    wq_cp.wait()
    q = jnp.dot(xn, wq_v[...], preferred_element_type=f32).astype(bf16)
    for h in range(H):
        q_v[h] = q[:, h * Dh:(h + 1) * Dh]

    x1 = xn.astype(f32)
    w3_cp.wait()
    a = lax.dot_general(_layernorm(x1).astype(bf16), w3_v[...],
                        (((1,), (1,)), ((), ())), preferred_element_type=f32)
    a = jax.nn.gelu(a, approximate=True).astype(bf16)
    w4_cp.wait()
    y = x1 + jnp.dot(a, w4_v[...], preferred_element_type=f32)
    g = y * jax.nn.sigmoid(y)

    scale = Dh ** -0.5

    def head(h, _):
        k_copy(h).wait()
        if depth < H:
            @pl.when(h + depth < H)
            def _():
                k_copy(h + depth).start()
        s = lax.dot_general(q_v[h], k_v[h], (((1,), (1,)), ((), ())),
                            preferred_element_type=f32) * scale
        m = jnp.max(s, axis=-1, keepdims=True)
        p = jnp.exp(s - m)
        l = jnp.sum(p, axis=-1, keepdims=True)
        v_copy(h).wait()
        if depth < H:
            @pl.when(h + depth < H)
            def _():
                v_copy(h + depth).start()
        o = jnp.dot(p.astype(bf16), v_v[h], preferred_element_type=f32)
        att_v[h] = (o / l).astype(bf16)

    lax.fori_loop(0, H, head, None)

    wo_cp.wait()
    att = jnp.concatenate([att_v[h] for h in range(H)], axis=-1)
    s_out = jnp.dot(att, wo_v[...], preferred_element_type=f32)
    o_ref[...] = (x + s_out * g).astype(o_ref.dtype)


@jax.jit
def pallas_recurrent_scan__sliding_block_cached__mixer_s_mlp__decode_kernel(
    A_x: jax.Array,
    A_k_cache: jax.Array,
    A_v_cache: jax.Array,
    A_wq: jax.Array,
    A_wo: jax.Array,
    B_x: jax.Array,
    B_w1: jax.Array,
    B_w2: jax.Array,
    B_w3: jax.Array,
    B_w4: jax.Array,
):
    B, Sq, D = A_x.shape
    _, H, Sk, Dh = A_k_cache.shape
    F = B_w3.shape[1]
    assert B == 1 and Sq == 1 and A_wq.shape[1] == H * Dh
    W = min(4096, max(256, Sk // 4))
    dt = A_x.dtype
    hbm = pl.BlockSpec(memory_space=pl.ANY)
    out = pl.pallas_call(
        functools.partial(_kernel, H=H, Dh=Dh, Sk=Sk, W=W, depth=4),
        in_specs=[hbm] * 7,
        out_specs=pl.BlockSpec(memory_space=pltpu.VMEM),
        out_shape=jax.ShapeDtypeStruct((Sq, D), dt),
        scratch_shapes=[
            pltpu.VMEM((Sq, D), dt),
            pltpu.VMEM((D, H * Dh), dt),
            pltpu.VMEM((H * Dh, D), dt),
            pltpu.VMEM((F, D), dt),
            pltpu.VMEM((F, D), dt),
            pltpu.VMEM((H, W, Dh), dt),
            pltpu.VMEM((H, W, Dh), dt),
            pltpu.VMEM((H, Sq, Dh), dt),
            pltpu.VMEM((H, Sq, Dh), dt),
            pltpu.SemaphoreType.DMA((5,)),
            pltpu.SemaphoreType.DMA((H,)),
            pltpu.SemaphoreType.DMA((H,)),
        ],
        compiler_params=pltpu.CompilerParams(
            vmem_limit_bytes=100 * 1024 * 1024),
    )(A_x.reshape(Sq, D), A_k_cache, A_v_cache, A_wq, A_wo, B_w3.T, B_w4)
    return out.reshape(B, Sq, D)
```

```python
import functools

import jax
import jax.numpy as jnp
from jax import lax
import jax.experimental.pallas as pl
import jax.experimental.pallas.tpu as pltpu

_EPS = 1e-5
_NT = (((1,), (1,)), ((), ()))


def _layernorm(x):
    m = jnp.mean(x, axis=-1, keepdims=True)
    d = x - m
    v = jnp.mean(d * d, axis=-1, keepdims=True)
    return d * lax.rsqrt(v + _EPS)


def _ranges(sizes):
    out, start = [], 0
    for n in sizes:
        out.append((start, n))
        start += n
    return out


def _kernel(x_hbm, k_hbm, v_hbm, wq_hbm, wo_hbm, w3t_hbm, w4_hbm, o_ref,
            x_v, wq_v, wo_v, w3t_v, w4_v, k_v, v_v, q_v, p_v, att_v, g_v, acc_v,
            sems, *, H, Dh, Sk, W, v_chunks, wo_chunks):
    bf16, f32 = jnp.bfloat16, jnp.float32
    win = pl.ds(Sk - W, W)
    v_rng, wo_rng = _ranges(v_chunks), _ranges(wo_chunks)

    pairs = [(x_hbm, x_v), (wq_hbm, wq_v), (k_hbm.at[0, :, win, :], k_v),
             (w3t_hbm, w3t_v), (w4_hbm, w4_v)]
    pairs += [(v_hbm.at[0, pl.ds(s, n), win, :], v_v.at[pl.ds(s, n)])
              for s, n in v_rng]
    pairs += [(wo_hbm.at[pl.ds(s * Dh, n * Dh), :],
               wo_v.at[pl.ds(s * Dh, n * Dh), :]) for s, n in wo_rng]
    copies = [pltpu.make_async_copy(src, dst, sems.at[i])
              for i, (src, dst) in enumerate(pairs)]
    for c in copies:
        c.start()
    pending = iter(copies)

    def wait_next():
        next(pending).wait()

    wait_next()
    xn = _layernorm(x_v[...].astype(f32)).astype(bf16)

    wait_next()
    q = jnp.dot(xn, wq_v[...], preferred_element_type=f32).astype(bf16)
    for h in range(H):
        q_v[h] = q[:, h * Dh:(h + 1) * Dh]

    def probs(h, _):
        s = lax.dot_general(q_v[h], k_v[h], _NT, preferred_element_type=f32)
        s = s * (Dh ** -0.5)
        e = jnp.exp(s - jnp.max(s, axis=-1, keepdims=True))
        p_v[h] = (e / jnp.sum(e, axis=-1, keepdims=True)).astype(bf16)

    wait_next()
    lax.fori_loop(0, H, probs, None)

    x1 = xn.astype(f32)
    wait_next()
    a = lax.dot_general(_layernorm(x1).astype(bf16), w3t_v[...], _NT,
                        preferred_element_type=f32)
    a = jax.nn.gelu(a, approximate=True).astype(bf16)
    wait_next()
    y = x1 + jnp.dot(a, w4_v[...], preferred_element_type=f32)
    g_v[...] = y * jax.nn.sigmoid(y)

    def weighted_sum(h, _):
        att_v[h] = jnp.dot(p_v[h], v_v[h],
                           preferred_element_type=f32).astype(bf16)

    for s, n in v_rng:
        wait_next()
        lax.fori_loop(s, s + n, weighted_sum, None)

    for i, (s, n) in enumerate(wo_rng):
        att = jnp.concatenate([att_v[h] for h in range(s, s + n)], axis=-1)
        wait_next()
        acc = jnp.dot(att, wo_v[pl.ds(s * Dh, n * Dh), :],
                      preferred_element_type=f32)
        if i > 0:
            acc = acc_v[...] + acc
        if i + 1 < len(wo_rng):
            acc_v[...] = acc
    o_ref[...] = (x_v[...].astype(f32) + acc * g_v[...]).astype(o_ref.dtype)


@jax.jit
def pallas_recurrent_scan__sliding_block_cached__mixer_s_mlp__decode_kernel(
    A_x: jax.Array,
    A_k_cache: jax.Array,
    A_v_cache: jax.Array,
    A_wq: jax.Array,
    A_wo: jax.Array,
    B_x: jax.Array,
    B_w1: jax.Array,
    B_w2: jax.Array,
    B_w3: jax.Array,
    B_w4: jax.Array,
):
    B, Sq, D = A_x.shape
    _, H, Sk, Dh = A_k_cache.shape
    F = B_w3.shape[1]
    assert B == 1 and Sq == 1 and H == 32 and A_wq.shape[1] == H * Dh
    W = min(4096, max(256, Sk // 4))
    dt = A_x.dtype
    v_chunks, wo_chunks = (24, 8), (25, 5, 2)
    out = pl.pallas_call(
        functools.partial(_kernel, H=H, Dh=Dh, Sk=Sk, W=W,
                          v_chunks=v_chunks, wo_chunks=wo_chunks),
        in_specs=[pl.BlockSpec(memory_space=pl.ANY)] * 7,
        out_specs=pl.BlockSpec(memory_space=pltpu.VMEM),
        out_shape=jax.ShapeDtypeStruct((Sq, D), dt),
        scratch_shapes=[
            pltpu.VMEM((Sq, D), dt),
            pltpu.VMEM((D, H * Dh), dt),
            pltpu.VMEM((H * Dh, D), dt),
            pltpu.VMEM((F, D), dt),
            pltpu.VMEM((F, D), dt),
            pltpu.VMEM((H, W, Dh), dt),
            pltpu.VMEM((H, W, Dh), dt),
            pltpu.VMEM((H, Sq, Dh), dt),
            pltpu.VMEM((H, Sq, W), dt),
            pltpu.VMEM((H, Sq, Dh), dt),
            pltpu.VMEM((Sq, D), jnp.float32),
            pltpu.VMEM((Sq, D), jnp.float32),
            pltpu.SemaphoreType.DMA((5 + len(v_chunks) + len(wo_chunks),)),
        ],
        compiler_params=pltpu.CompilerParams(
            vmem_limit_bytes=100 * 1024 * 1024,
            disable_bounds_checks=True,
            disable_semaphore_checks=True,
            skip_device_barrier=True,
        ),
    )(A_x.reshape(Sq, D), A_k_cache, A_v_cache, A_wq, A_wo, B_w3.T, B_w4)
    return out.reshape(B, Sq, D)
```
